```python
import os as _os
_os.environ.setdefault("JAX_PLATFORMS", "cpu")
import jax
import jax.numpy as jnp

def _softmax(x, axis=-1):
    return jax.nn.softmax(x, axis=axis)
def _gelu(x):
    return jax.nn.gelu(x, approximate=True)
def _silu(x):
    return jax.nn.silu(x)
def _sigmoid(x):
    return jax.nn.sigmoid(x)
def _layernorm(x, axis=-1, eps=1e-5):
    m = jnp.mean(x, axis=axis, keepdims=True)
    v = jnp.var(x, axis=axis, keepdims=True)
    return (x - m) / jnp.sqrt(v + eps)
def _scatter_add(tgt, idx, src, axis=0):
    return tgt.at[idx].add(src)
def _segment_sum(src, seg, n):
    return jax.ops.segment_sum(src, seg, n)
class _Rng:
    def __init__(self, key):
        self._k = key
    def _next(self):
        self._k, sub = jax.random.split(self._k)
        return sub
    def normal(self, shape):
        return jax.random.normal(self._next(), shape, dtype=jnp.bfloat16)
    def randint(self, lo, hi, shape):
        return jax.random.randint(self._next(), shape, lo, hi, dtype=jnp.int32)
    def uniform(self, shape, lo=0.0, hi=1.0):
        return jax.random.uniform(self._next(), shape, jnp.bfloat16, lo, hi)
    def permutation(self, n):
        return jax.random.permutation(self._next(), n)


kernel_name = 'standalone__mha_block_cached__near_ridge'

def setup_inputs():
    _rng = _Rng(jax.random.key(int.from_bytes(__import__("os").urandom(4), "little")))
    _w = (lambda a: (lambda t: t.astype(jnp.bfloat16) if jnp.issubdtype(t.dtype, jnp.floating) else t)(jnp.asarray(a)))
    B, Sq, D = 8, 144, 448
    H, Sk, Dh = 16, 2048, 256
    return {
        "x": _w((lambda *s: _rng.normal(s) * 0.8)(B, Sq, D)),
        "k_cache": _w((lambda *s: _rng.normal(s) * 0.8)(B, H, Sk, Dh)),
        "v_cache": _w((lambda *s: _rng.normal(s) * 0.05)(B, H, Sk, Dh)),
        "wq": _w((lambda *s: _rng.normal(s) * 0.8)(D, H * Dh) * (D ** -0.5)),
        "wo": _w((lambda *s: _rng.normal(s) * 0.05)(H * Dh, D) * ((H * Dh) ** -0.5)),
    }

def reference(x, k_cache, v_cache, wq, wo):
    B, Sq, D = x.shape
    H, Dh = 16, 256
    q = (lambda x, *d: x.transpose(*d))((x @ wq).reshape(B, Sq, H, Dh), 0, 2, 1, 3)
    scores = jnp.einsum("bhqd,bhkd->bhqk", q, k_cache) * (Dh ** -0.5)
    p = _softmax(scores, axis=-1)
    o = jnp.einsum("bhqk,bhkd->bhqd", p, v_cache)
    return (lambda x, *d: x.transpose(*d))(o, 0, 2, 1, 3).reshape(B, Sq, H * Dh) @ wo
```

```python
import jax
import jax.numpy as jnp
from jax import lax
import jax.experimental.pallas as pl
import jax.experimental.pallas.tpu as pltpu

_ROWS = 96
_LA0 = 23
_QD = 26


def _chunks(total, size):
    return [(o, min(size, total - o)) for o in range(0, total, size)]


@jax.jit
def pallas_standalone__mha_block_cached__near_ridge_kernel(
    x: jax.Array,
    k_cache: jax.Array,
    v_cache: jax.Array,
    wq: jax.Array,
    wo: jax.Array,
):
    B, SQ, D = x.shape
    _, H, SK, DH = k_cache.shape
    NSTEP = B * H
    bf16, f32 = jnp.bfloat16, jnp.float32

    ch = _chunks(SK, _ROWS)
    n = len(ch)
    la0, la1 = _LA0, _LA0 + _QD
    nk = 1 + -(-la0 // n)
    nv = 1 + -(-la1 // n)

    def kernel_function(x_hbm, k_hbm, v_hbm, wq_hbm, wo_hbm, out_hbm,
                        xbuf, wqbuf, wobuf, kbuf, vbuf, acc, obuf,
                        ksem, vsem, wsem, osem):

        def k_copy(step, c):
            o, r = ch[c]
            slot = step % nk
            return pltpu.make_async_copy(
                k_hbm.at[step, pl.ds(o, r)], kbuf.at[slot, pl.ds(o, r)], ksem.at[slot])

        def v_copy(step, c):
            o, r = ch[c]
            slot = step % nv
            return pltpu.make_async_copy(
                v_hbm.at[step, pl.ds(o, r)], vbuf.at[slot, pl.ds(o, r)], vsem.at[slot])

        s0, s1 = [], []
        for b in range(B):
            for o, r in _chunks(SQ, SQ // 2):
                (s0 if b < B // 2 else s1).append(pltpu.make_async_copy(
                    x_hbm.at[b, pl.ds(o, r)], xbuf.at[b, pl.ds(o, r)], wsem.at[0]))
        for r in range(0, D, 8):
            s0.append(pltpu.make_async_copy(
                wq_hbm.at[pl.ds(r, 8)], wqbuf.at[pl.ds(r, 8)], wsem.at[1]))
            s1.append(pltpu.make_async_copy(
                wo_hbm.at[pl.ds(r, 8)], wobuf.at[pl.ds(r, 8)], wsem.at[2]))
        s0 += [k_copy(g // n, g % n) for g in range(la0)]
        s1 += [v_copy(g // n, g % n) for g in range(la1)]
        for c in s1[:_QD]:
            c.start(priority=1)
        for c0, c1 in zip(s0, s1[_QD:]):
            c0.start(priority=0)
            c1.start(priority=1)
        acc[...] = jnp.zeros(acc.shape, f32)
        pltpu.make_async_copy(xbuf, xbuf, wsem.at[0]).wait()
        pltpu.make_async_copy(wqbuf, wqbuf, wsem.at[1]).wait()
        pltpu.make_async_copy(wobuf, wobuf, wsem.at[2]).wait()

        items = []
        for j in range(n):
            items.append((k_copy, 0, (la0 + j) // n, (la0 + j) % n))
            items.append((v_copy, 1, (la1 + j) // n, (la1 + j) % n))
        maxoff = max(it[2] for it in items)

        def issue(i):
            @pl.when(i + maxoff < NSTEP)
            def _():
                for mk, prio, off, c in items:
                    mk(i + off, c).start(priority=prio)

            @pl.when(i + maxoff >= NSTEP)
            def _():
                for mk, prio, off, c in items:
                    @pl.when(i + off < NSTEP)
                    def _():
                        mk(i + off, c).start(priority=prio)

        def body(i, carry):
            b = i // H
            h = i % H
            ks = i % nk
            vs = i % nv
            issue(i)

            @pl.when(i == NSTEP - 1)
            def _():
                pltpu.make_async_copy(obuf.at[pl.ds(0, B - 1)], out_hbm.at[pl.ds(0, B - 1)],
                                      osem.at[0]).start()

            pltpu.make_async_copy(kbuf.at[ks], kbuf.at[ks], ksem.at[ks]).wait()
            pltpu.make_async_copy(vbuf.at[vs], vbuf.at[vs], vsem.at[vs]).wait()

            col = pl.multiple_of(h * DH, DH)
            q = jnp.dot(xbuf[b], wqbuf[:, pl.ds(col, DH)], preferred_element_type=f32)
            q = (q * (DH ** -0.5)).astype(bf16)
            s = lax.dot_general(q, kbuf[ks], (((1,), (1,)), ((), ())),
                                preferred_element_type=f32)
            m = jnp.max(s, axis=-1, keepdims=True)
            p = jnp.exp(s - m)
            l = jnp.sum(p, axis=-1, keepdims=True)
            o = jnp.dot(p.astype(bf16), vbuf[vs], preferred_element_type=f32)
            o = (o / l).astype(bf16)
            y = lax.dot_general(o, wobuf[:, pl.ds(col, DH)], (((1,), (1,)), ((), ())),
                                preferred_element_type=f32)
            acc[...] += y

            @pl.when(h == H - 1)
            def _():
                obuf[b] = acc[...].astype(bf16)
                acc[...] = jnp.zeros(acc.shape, f32)

            return carry

        lax.fori_loop(0, NSTEP, body, 0)
        last = pltpu.make_async_copy(obuf.at[B - 1], out_hbm.at[B - 1], osem.at[1])
        last.start()
        pltpu.make_async_copy(obuf.at[pl.ds(0, B - 1)], out_hbm.at[pl.ds(0, B - 1)],
                              osem.at[0]).wait()
        last.wait()

    hbm = pl.BlockSpec(memory_space=pltpu.MemorySpace.HBM)
    return pl.pallas_call(
        kernel_function,
        in_specs=[hbm] * 5,
        out_specs=hbm,
        out_shape=jax.ShapeDtypeStruct((B, SQ, D), x.dtype),
        scratch_shapes=[
            pltpu.VMEM((B, SQ, D), bf16),
            pltpu.VMEM((D, H * DH), bf16),
            pltpu.VMEM((D, H * DH), bf16),
            pltpu.VMEM((nk, SK, DH), bf16),
            pltpu.VMEM((nv, SK, DH), bf16),
            pltpu.VMEM((SQ, D), f32),
            pltpu.VMEM((B, SQ, D), bf16),
            pltpu.SemaphoreType.DMA((nk,)),
            pltpu.SemaphoreType.DMA((nv,)),
            pltpu.SemaphoreType.DMA((3,)),
            pltpu.SemaphoreType.DMA((2,)),
        ],
        compiler_params=pltpu.CompilerParams(
            vmem_limit_bytes=64 * 1024 * 1024, disable_bounds_checks=True),
    )(x, k_cache.reshape(NSTEP, SK, DH), v_cache.reshape(NSTEP, SK, DH), wq, wo.T)
```

```python
import functools
import jax
import jax.numpy as jnp
from jax import lax
import jax.experimental.pallas as pl
import jax.experimental.pallas.tpu as pltpu

B, SQ, D = 8, 144, 448
H, SK, DH = 16, 2048, 256
NSTEP = B * H
bf16, f32 = jnp.bfloat16, jnp.float32
NT = (((1,), (1,)), ((), ()))
TPS = SK // 8 * 2

def chunks(total, size):
    return [(o, min(size, total - o)) for o in range(0, total, size)]

def rr(*streams):
    streams = [list(s) for s in streams]
    out = []
    while any(streams):
        for s in streams:
            if s:
                out.append(s.pop(0))
    return out

def merge(bl, al, f):
    nb = len(bl)
    na_early = int(round(nb * f)) - nb
    out = []
    bi = ai = 0
    gb = [bl[j:j + 2] for j in range(0, nb, 2)]
    ga = [al[j:j + 2] for j in range(0, len(al), 2)]
    ne = na_early // 2
    k = 0
    for j, g in enumerate(gb):
        out += g
        want = ((j + 1) * ne) // len(gb)
        while k < want:
            out += ga[k]; k += 1
    for g in ga[k:]:
        out += g
    return out

def make(delta=-3, px=45, py=59, qd=26, fs=(1.72, 1.44, 1.16, 1.0), cu=14.2, wafter=True, compute=True,
         wcols=2048, xrows=48, skip_w=False, nslot=None, ws=4, verbose=False):
    e = [0] + [16 * k + delta for k in range(1, 32)] + [TPS]
    ch = [(e[k], e[k + 1] - e[k]) for k in range(32)]
    grp = [1 if (k // 8) % 2 == 0 else 0 for k in range(32)]
    up = lambda t: (t + 1) // 2
    a_lo = (up(e[8]), e[16] // 2)
    na_hi = 128 - (a_lo[1] - a_lo[0])
    a_hi = (256 - na_hi, 256)
    assert a_hi[0] >= up(e[24])
    a_rg = [a_lo, a_hi]
    b_rg = [(0, a_lo[0]), (a_lo[1], a_hi[0])]
    regions = {0: [(e[8], e[16]), (e[24], TPS)], 1: [(0, e[8]), (e[16], e[24])]}

    A = lambda i: rr([(i, k) for k in range(8, 16)], [(i, k) for k in range(24, 32)])
    Bq = lambda i: rr([(i, k) for k in range(0, 8)], [(i, k) for k in range(16, 24)])
    L = list(A(0))
    for i in range(NSTEP - 1):
        j = i - (NSTEP - 1 - len(fs))
        L += merge(Bq(i), A(i + 1), fs[j] if j >= 0 else 2.0)
    L += Bq(NSTEP - 1)
    G = len(L)
    assert G == NSTEP * 32 and len(set(L)) == G
    done = {}
    for pos, (i, k) in enumerate(L):
        done[(i, grp[k])] = pos + 1
    T = (qd + 1) // 2
    S0 = [("k",) + d for d in L[:G - T]]
    S1 = [("v",) + d for d in L[:G - T]]
    for d in L[G - T:]:
        S1 += [("k",) + d, ("v",) + d]
    npairs = max(len(S0), len(S1) - qd)
    pair = lambda t: (S0[t] if t < len(S0) else None, S1[t + qd] if t + qd < len(S1) else None)
    lax_, lay_ = px - cu, py - 2 * cu
    lim = {}
    t = 0.0
    first_irr = NSTEP - 1 - len(fs)
    for i in range(NSTEP):
        E = 16 + 32 * i
        for u in (0, 1):
            reg = E + (px if u == 0 else py)
            sim = int(round(t + (lax_ if u == 0 else lay_)))
            lim[(i, u)] = min(npairs, reg if i <= first_irr else min(reg, sim))
            t = max(t, done[(i, u)]) + cu
    order = [(i, u) for i in range(NSTEP) for u in (0, 1)]
    start0 = 16 + py - 32
    prev = start0
    bursts = {}
    for key in order:
        lim[key] = max(lim[key], prev)
        bursts[key] = [pair(t_) for t_ in range(prev, lim[key])]
        prev = lim[key]
    assert prev == npairs
    rel = lambda key: [tuple(None if d is None else (d[0], d[1] - key[0], d[2]) for d in p) for p in bursts[key]]
    regpat = {u: rel((1, u)) for u in (0, 1)}
    nreg = 0
    while all(rel((nreg, u)) == regpat[u] for u in (0, 1)):
        nreg += 1
    issued = set(S1[:qd]) | {d for t_ in range(start0) for d in pair(t_) if d}
    need_slots = 1 + max(d[1] for d in issued)
    for key in order:
        for p in bursts[key]:
            for d in p:
                if d:
                    issued.add(d)
                    need_slots = max(need_slots, d[1] - key[0] + 1)
        for kind in "kv":
            for k in range(32):
                if grp[k] == key[1]:
                    assert (kind, key[0], k) in issued, (key, kind, k)
    ns = nslot or need_slots
    assert ns >= need_slots
    if verbose:
        print("nreg", nreg, "slots", need_slots, "burst sizes", [len(bursts[k]) for k in order[2 * nreg - 4:]])

    def kern(x_hbm, k_hbm, v_hbm, wq_hbm, wo_hbm, out_hbm,
             xbuf, wqbuf, wobuf, kbuf, vbuf, acc, obuf, qbuf, opbuf, sem, osem):

        def sem_of(kind, slot, g):
            return sem.at[3 + (0 if kind == "k" else 2 * ns) + 2 * slot + g]

        def kv_copy(kind, step, k):
            o, r = ch[k]
            slot = step % ns
            src, dst = (k_hbm, kbuf) if kind == "k" else (v_hbm, vbuf)
            return pltpu.make_async_copy(src.at[step, pl.ds(o, r)], dst.at[slot, pl.ds(o, r)], sem_of(kind, slot, grp[k]))

        s0, s1 = [], []
        if not skip_w:
            xs = [[pltpu.make_async_copy(x_hbm.at[b, pl.ds(o, r)], xbuf.at[b, pl.ds(o, r)], sem.at[0])
                   for o, r in chunks(SQ, xrows)] for b in range(B)]
            def wstreams(src, dst, sm):
                per = D // 8 // ws
                return [[pltpu.make_async_copy(src.at[pl.ds(r * 8, 8), pl.ds(co, cw)], dst.at[pl.ds(r * 8, 8), pl.ds(co, cw)], sm)
                         for r in range(w * per, (w + 1) * per) for co, cw in chunks(H * DH, wcols)] for w in range(ws)]
            s0 = rr(sum(xs[:4], []), *wstreams(wq_hbm, wqbuf, sem.at[1]))
            s1 = rr(sum(xs[4:], []), *wstreams(wo_hbm, wobuf, sem.at[2]))
        s0 += [kv_copy(*d) for d in S0[:start0]]
        s1 += [kv_copy(*d) for d in S1[:start0 + qd]]
        for c in s1[:qd]:
            c.start(priority=1)
        for c0, c1 in zip(s0, s1[qd:]):
            c0.start(priority=0)
            c1.start(priority=1)
        acc[...] = jnp.zeros(acc.shape, f32)
        opbuf[...] = jnp.zeros(opbuf.shape, bf16)
        if not skip_w:
            pltpu.make_async_copy(xbuf, xbuf, sem.at[0]).wait()
            pltpu.make_async_copy(wqbuf, wqbuf, sem.at[1]).wait()
            pltpu.make_async_copy(wobuf, wobuf, sem.at[2]).wait()

        def qproj(i):
            b = i // H
            col = pl.multiple_of((i % H) * DH, DH)
            q = jnp.dot(xbuf[b], wqbuf[:, pl.ds(col, DH)], preferred_element_type=f32)
            return (q * (DH ** -0.5)).astype(bf16)

        def oproj(h):
            col = pl.multiple_of(h * DH, DH)
            return lax.dot_general(opbuf[...], wobuf[:, pl.ds(col, DH)], NT, preferred_element_type=f32)

        qbuf[...] = qproj(0)

        def issue(i, u):
            @pl.when(i < nreg)
            def _():
                for p in regpat[u]:
                    for prio, d in enumerate(p):
                        kv_copy(d[0], i + d[1], d[2]).start(priority=prio)

            @pl.when(i >= nreg)
            def _():
                for ii in range(nreg, NSTEP):
                    if not bursts[(ii, u)]:
                        continue
                    @pl.when(i == ii)
                    def _():
                        for p in bursts[(ii, u)]:
                            for prio, d in enumerate(p):
                                if d is not None:
                                    kv_copy(*d).start(priority=prio)

        def wait(slot, g):
            for kind, buf in (("k", kbuf), ("v", vbuf)):
                for lo, hi in regions[g]:
                    r = buf.at[slot, pl.ds(lo, hi - lo)]
                    pltpu.make_async_copy(r, r, sem_of(kind, slot, g)).wait()

        def load(buf, slot, rgs):
            t = jnp.concatenate([buf[slot, pl.ds(2 * lo, 2 * (hi - lo))] for lo, hi in rgs], axis=0)
            t = t.reshape(128, 2, 8, 128)
            return jnp.concatenate([t[:, 0].reshape(1024, 128), t[:, 1].reshape(1024, 128)], axis=1)

        def bulk_out():
            return pltpu.make_async_copy(obuf.at[pl.ds(0, B - 1)], out_hbm.at[pl.ds(0, B - 1)], osem.at[0])

        def body(i, carry):
            b = i // H
            h = i % H
            slot = i % ns
            issue(i, 0)
            wait(slot, 0)
            if compute:
                q = qbuf[...]
                s = lax.dot_general(q, load(kbuf, slot, a_rg), NT, preferred_element_type=f32)
                acc[...] += oproj((h + H - 1) % H)
                m0 = jnp.max(s, axis=-1, keepdims=True)
                p = jnp.exp(s - m0)
                l0 = jnp.sum(p, axis=-1, keepdims=True)
                o0 = jnp.dot(p.astype(bf16), load(vbuf, slot, a_rg), preferred_element_type=f32)

            @pl.when(jnp.logical_and(h == 0, i > 0))
            def _():
                obuf[b - 1] = acc[...].astype(bf16)
                acc[...] = jnp.zeros(acc.shape, f32)

            issue(i, 1)
            if not wafter:
                pl.when(i == NSTEP - 1)(lambda: bulk_out().start())
            wait(slot, 1)
            if wafter:
                pl.when(i == NSTEP - 1)(lambda: bulk_out().start())
            if compute:
                q = qbuf[...]
                s = lax.dot_general(q, load(kbuf, slot, b_rg), NT, preferred_element_type=f32)
                qbuf[...] = qproj(jnp.minimum(i + 1, NSTEP - 1))
                m = jnp.maximum(m0, jnp.max(s, axis=-1, keepdims=True))
                a = jnp.exp(m0 - m)
                p = jnp.exp(s - m)
                l = a * l0 + jnp.sum(p, axis=-1, keepdims=True)
                o = a * o0 + jnp.dot(p.astype(bf16), load(vbuf, slot, b_rg), preferred_element_type=f32)
                opbuf[...] = (o / l).astype(bf16)
            return carry

        lax.fori_loop(0, NSTEP, body, 0)
        obuf[B - 1] = (acc[...] + oproj(H - 1)).astype(bf16)
        last = pltpu.make_async_copy(obuf.at[B - 1], out_hbm.at[B - 1], osem.at[1])
        last.start()
        bulk_out().wait()
        last.wait()

    def tiles(a):
        return a.reshape(NSTEP, SK // 8, 8, 2, 128).transpose(0, 1, 3, 2, 4).reshape(NSTEP, TPS, 8, 128)

    @jax.jit
    def f(x, k_cache, v_cache, wq, wo):
        hbm = pl.BlockSpec(memory_space=pltpu.MemorySpace.HBM)
        return pl.pallas_call(
            kern,
            in_specs=[hbm] * 5,
            out_specs=hbm,
            out_shape=jax.ShapeDtypeStruct((B, SQ, D), bf16),
            scratch_shapes=[
                pltpu.VMEM((B, SQ, D), bf16), pltpu.VMEM((D, H * DH), bf16), pltpu.VMEM((D, H * DH), bf16),
                pltpu.VMEM((ns, TPS, 8, 128), bf16), pltpu.VMEM((ns, TPS, 8, 128), bf16),
                pltpu.VMEM((SQ, D), f32), pltpu.VMEM((B, SQ, D), bf16),
                pltpu.VMEM((SQ, DH), bf16), pltpu.VMEM((SQ, DH), bf16),
                pltpu.SemaphoreType.DMA((3 + 4 * ns,)), pltpu.SemaphoreType.DMA((2,)),
            ],
            compiler_params=pltpu.CompilerParams(vmem_limit_bytes=64 * 1024 * 1024, disable_bounds_checks=True),
        )(x, tiles(k_cache), tiles(v_cache), wq, wo.T)
    return f


_f = make(**OPQ)


@jax.jit
def pallas_standalone__mha_block_cached__near_ridge_kernel(x, k_cache, v_cache, wq, wo):
    return _f(x, k_cache, v_cache, wq, wo)
```

```python
import jax
import jax.numpy as jnp
from jax import lax
import jax.experimental.pallas as pl
import jax.experimental.pallas.tpu as pltpu

_CT = 16
_DELTA = -3
_QD = 26
_PX, _PY = 41, 57
_LA_END = 31
_CU = 14.7
_FS = (1.75, 1.625, 1.5, 1.375, 1.25, 1.0, 1.0)
_VROT = 2
_VTAIL = 10
_WS = 4
_XROWS = 32

_NT = (((1,), (1,)), ((), ()))


def _rr(*streams):
    streams = [list(s) for s in streams]
    out = []
    while any(streams):
        for s in streams:
            if s:
                out.append(s.pop(0))
    return out


def _merge(bl, al, f):
    gb = [bl[j:j + 2] for j in range(0, len(bl), 2)]
    ga = [al[j:j + 2] for j in range(0, len(al), 2)]
    ne = (int(round(len(bl) * f)) - len(bl)) // 2
    out, k = [], 0
    for j, g in enumerate(gb):
        out += g
        while k < ((j + 1) * ne) // len(gb):
            out += ga[k]
            k += 1
    for g in ga[k:]:
        out += g
    return out


def _schedule(nstep):
    last = nstep - 1
    grp = [1 - (k // 8) % 2 for k in range(32)]
    ua = lambda i: _rr([(i, k) for k in range(8, 16)], [(i, k) for k in range(24, 32)])
    ub = lambda i: _rr([(i, k) for k in range(0, 8)], [(i, k) for k in range(16, 24)])
    kd = lambda l: [("k",) + d for d in l]
    vd = lambda l: [("v", i, k // 8 * 8 + (k + _VROT) % 8) for i, k in l]

    first_irr = last - len(_FS)
    seq = ua(0)
    for i in range(last):
        seq += _merge(ub(i), ua(i + 1), _FS[i - first_irr] if i >= first_irr else 2.0)
    order = _rr(kd(seq), vd(seq))
    tk, tv, nv = kd(ub(last)), vd(ub(last)), 0
    for j, d in enumerate(tk):
        while nv < ((j + 1) * (len(tv) - _VTAIL)) // len(tk):
            order.append(tv[nv])
            nv += 1
        order.append(d)
    order += tv[nv:]
    assert len(set(order)) == len(order) == nstep * 64

    s0 = order[:len(order) - _QD:2]
    s1 = order[1:len(order) - _QD:2] + order[len(order) - _QD:]
    pairs = list(zip(s0, s1[_QD:]))
    assert len(s0) == len(s1) - _QD

    done = {}
    for pos, (_, i, k) in enumerate(order):
        done[(i, grp[k])] = (pos + 1) / 2
    npro = 16 + _PY - 32
    prev, t, bursts = npro, 0.0, {}
    for i in range(nstep):
        for u in (0, 1):
            lim = 16 + 32 * i + (_PX, _PY)[u]
            if i > first_irr:
                lim = min(lim, int(round(t + _LA_END)))
            lim = len(pairs) if i == last else max(prev, min(lim, len(pairs)))
            bursts[(i, u)] = pairs[prev:lim]
            prev = lim
            t = max(t, done[(i, u)]) + _CU

    rel = lambda i, u: [tuple((c, j - i, k) for c, j, k in p) for p in bursts[(i, u)]]
    regular = [rel(1, 0), rel(1, 1)]
    nreg = 0
    while [rel(nreg, 0), rel(nreg, 1)] == regular:
        nreg += 1

    issued = set(s1[:_QD]) | {d for p in pairs[:npro] for d in p}
    nslot = 1 + max(d[1] for d in issued)
    for i in range(nstep):
        for u in (0, 1):
            for p in bursts[(i, u)]:
                issued.update(p)
                nslot = max(nslot, 1 + max(d[1] for d in p) - i)
            assert all((c, i, k) in issued for c in "kv" for k in range(32) if grp[k] == u)
    return grp, s0[:npro], s1[:npro + _QD], bursts, regular, nreg, nslot


@jax.jit
def pallas_standalone__mha_block_cached__near_ridge_kernel(
    x: jax.Array,
    k_cache: jax.Array,
    v_cache: jax.Array,
    wq: jax.Array,
    wo: jax.Array,
):
    B, SQ, D = x.shape
    _, H, SK, DH = k_cache.shape
    assert (SK, DH) == (2048, 256) and D % (8 * _WS) == 0
    bf16, f32 = jnp.bfloat16, jnp.float32
    NSTEP = B * H
    LAST = NSTEP - 1
    TPS = SK // 8 * 2
    WT = H * DH // 128
    SU = SK // 2

    edge = [0] + [_CT * k + _DELTA for k in range(1, 32)] + [TPS]
    a_lo = ((edge[8] + 1) // 2, edge[16] // 2)
    a_hi = (TPS // 2 - (SU // 8 - (a_lo[1] - a_lo[0])), TPS // 2)
    assert 2 * a_hi[0] >= edge[24]
    rowgroups = ([a_lo, a_hi], [(0, a_lo[0]), (a_lo[1], a_hi[0])])
    grp, pro0, pro1, bursts, regular, nreg, ns = _schedule(NSTEP)

    def kernel_function(x_hbm, k_hbm, v_hbm, wq_hbm, wo_hbm, out_hbm,
                        xbuf, wqbuf, wobuf, kbuf, vbuf, acc, obuf, qbuf, opbuf,
                        sem, osem):

        def kv_copy(kind, step, k):
            src, dst, base = (k_hbm, kbuf, 3) if kind == "k" else (v_hbm, vbuf, 3 + 2 * ns)
            slot = step % ns
            tiles = pl.ds(edge[k], edge[k + 1] - edge[k])
            return pltpu.make_async_copy(
                src.at[step, tiles], dst.at[slot, tiles], sem.at[base + 2 * slot + grp[k]])

        def start_pairs(pairs, step0=0):
            for pair in pairs:
                for prio, (kind, step, k) in enumerate(pair):
                    kv_copy(kind, step0 + step, k).start(priority=prio)

        def wait(kind, step, g):
            for k in range(32):
                if grp[k] == g:
                    kv_copy(kind, step, k).wait()

        def w_streams(src, dst, s):
            per = D // 8 // _WS * WT
            streams = []
            for w in range(_WS):
                t0, t1 = w * per, (w + 1) * per
                cuts = [t0] + [t for t in range(t0 + 1, t1) if (t - _DELTA) % _CT == 0] + [t1]
                visits = []
                for lo, hi in zip(cuts[:-1], cuts[1:]):
                    visits.append([])
                    while lo < hi:
                        nx = min(hi, (lo // WT + 1) * WT)
                        idx = (pl.ds(lo // WT * 8, 8), pl.ds(lo % WT * 128, (nx - lo) * 128))
                        visits[-1].append(pltpu.make_async_copy(src.at[idx], dst.at[idx], s))
                        lo = nx
                streams.append(visits)
            return streams

        def out_copy(lo, n, s):
            return pltpu.make_async_copy(
                obuf.at[pl.ds(lo, n)], out_hbm.at[pl.ds(lo, n)], osem.at[s])

        xs = []
        for b in range(B):
            for r in range(0, SQ, _XROWS):
                rows = pl.ds(r, min(_XROWS, SQ - r))
                xs.append([pltpu.make_async_copy(x_hbm.at[b, rows], xbuf.at[b, rows], sem.at[0])])
        s0 = sum(_rr(xs[:len(xs) // 2], *w_streams(wq_hbm, wqbuf, sem.at[1])), [])
        s1 = sum(_rr(xs[len(xs) // 2:], *w_streams(wo_hbm, wobuf, sem.at[2])), [])
        s0 += [kv_copy(*d) for d in pro0]
        s1 += [kv_copy(*d) for d in pro1]
        assert len(s0) == len(s1) - _QD
        for c in s1[:_QD]:
            c.start(priority=1)
        for c0, c1 in zip(s0, s1[_QD:]):
            c0.start(priority=0)
            c1.start(priority=1)
        acc[...] = jnp.zeros(acc.shape, f32)
        opbuf[...] = jnp.zeros(opbuf.shape, bf16)
        pltpu.make_async_copy(xbuf, xbuf, sem.at[0]).wait()
        pltpu.make_async_copy(wqbuf, wqbuf, sem.at[1]).wait()
        pltpu.make_async_copy(wobuf, wobuf, sem.at[2]).wait()

        def qproj(i):
            col = pl.multiple_of((i % H) * DH, DH)
            q = jnp.dot(xbuf[i // H], wqbuf[:, pl.ds(col, DH)], preferred_element_type=f32)
            return (q * (DH ** -0.5)).astype(bf16)

        def oproj(o, h):
            col = pl.multiple_of(h * DH, DH)
            return lax.dot_general(o, wobuf[:, pl.ds(col, DH)], _NT, preferred_element_type=f32)

        def load(buf, step, g):
            slot = step % ns
            t = jnp.concatenate(
                [buf[slot, pl.ds(2 * lo, 2 * (hi - lo))] for lo, hi in rowgroups[g]], axis=0)
            t = t.reshape(SU // 8, 2, 8, 128)
            return jnp.concatenate(
                [t[:, 0].reshape(SU, 128), t[:, 1].reshape(SU, 128)], axis=1)

        def scores(k):
            return lax.dot_general(qbuf[...], k, _NT, preferred_element_type=f32)

        def attend(s, v, state=None):
            m = jnp.max(s, axis=-1, keepdims=True)
            if state is not None:
                m = jnp.maximum(state[0], m)
                a = jnp.exp(state[0] - m)
            p = jnp.exp(s - m)
            l = jnp.sum(p, axis=-1, keepdims=True)
            o = jnp.dot(p.astype(bf16), v, preferred_element_type=f32)
            if state is not None:
                l = a * state[1] + l
                o = a * state[2] + o
            return m, l, o

        def issue(i, u):
            pl.when(i < nreg)(lambda: start_pairs(regular[u], i))

            def dispatch(steps):
                if len(steps) > 2:
                    mid = len(steps) // 2
                    lax.cond(i < steps[mid],
                             lambda: dispatch(steps[:mid]), lambda: dispatch(steps[mid:]))
                    return
                for j in steps:
                    lax.fori_loop(0, (i == j).astype(jnp.int32),
                                  lambda _, c, j=j: (start_pairs(bursts[(j, u)]), c)[1], 0)

            pl.when(i >= nreg)(
                lambda: dispatch([j for j in range(nreg, LAST) if bursts[(j, u)]]))

        qbuf[...] = qproj(0)

        def body(i, carry):
            h = i % H
            issue(i, 0)
            wait("k", i, 0)
            wait("v", i, 0)
            s = scores(load(kbuf, i, 0))
            acc[...] += oproj(opbuf[...], (h + H - 1) % H)
            state = attend(s, load(vbuf, i, 0))

            @pl.when(jnp.logical_and(h == 0, i > 0))
            def _():
                obuf[i // H - 1] = acc[...].astype(bf16)
                acc[...] = jnp.zeros(acc.shape, f32)

            issue(i, 1)
            wait("k", i, 1)
            wait("v", i, 1)
            s = scores(load(kbuf, i, 1))
            qbuf[...] = qproj(i + 1)
            _, l, o = attend(s, load(vbuf, i, 1), state)
            opbuf[...] = (o / l).astype(bf16)
            return carry

        lax.fori_loop(0, LAST, body, 0)

        def unit(g, state):
            k, v = load(kbuf, LAST, g), load(vbuf, LAST, g)
            s1_, s2_ = scores(k[:SU // 2]), scores(k[SU // 2:])
            return attend(s2_, v[SU // 2:], attend(s1_, v[:SU // 2], state))

        start_pairs(bursts[(LAST, 0)])
        acc[...] += oproj(opbuf[...], H - 2)
        wait("k", LAST, 0)
        wait("v", LAST, 0)
        state = unit(0, None)
        wait("k", LAST, 1)
        out_copy(0, B - 1, 0).start()
        wait("v", LAST, 1)
        _, l, o = unit(1, state)
        obuf[B - 1] = (acc[...] + oproj((o / l).astype(bf16), H - 1)).astype(bf16)
        out_copy(B - 1, 1, 1).start()
        out_copy(0, B - 1, 0).wait()
        out_copy(B - 1, 1, 1).wait()

    def tile_view(a):
        a = a.reshape(NSTEP, SK // 8, 8, 2, 128).transpose(0, 1, 3, 2, 4)
        return a.reshape(NSTEP, TPS, 8, 128)

    hbm = pl.BlockSpec(memory_space=pltpu.MemorySpace.HBM)
    return pl.pallas_call(
        kernel_function,
        in_specs=[hbm] * 5,
        out_specs=hbm,
        out_shape=jax.ShapeDtypeStruct((B, SQ, D), x.dtype),
        scratch_shapes=[
            pltpu.VMEM((B, SQ, D), bf16),
            pltpu.VMEM((D, H * DH), bf16),
            pltpu.VMEM((D, H * DH), bf16),
            pltpu.VMEM((ns, TPS, 8, 128), bf16),
            pltpu.VMEM((ns, TPS, 8, 128), bf16),
            pltpu.VMEM((SQ, D), f32),
            pltpu.VMEM((B, SQ, D), bf16),
            pltpu.VMEM((SQ, DH), bf16),
            pltpu.VMEM((SQ, DH), bf16),
            pltpu.SemaphoreType.DMA((3 + 4 * ns,)),
            pltpu.SemaphoreType.DMA((2,)),
        ],
        compiler_params=pltpu.CompilerParams(
            vmem_limit_bytes=48 * 1024 * 1024,
            disable_bounds_checks=True,
            disable_semaphore_checks=True,
        ),
    )(x, tile_view(k_cache), tile_view(v_cache), wq, wo.T)
```

```python
import jax
import jax.numpy as jnp
from jax import lax
import jax.experimental.pallas as pl
import jax.experimental.pallas.tpu as pltpu

_CT = 16
_PH = 13
_QD = 26
_PX, _PY = 40, 56
_LA_END = 28.6
_CU = 13.6
_FS = (1.75, 1.5, 1.25, 1.0, 1.0)
_VTAIL = 5
_WS = 4
_XROWS = 32

_EDGE = [0] + [_CT * k + _PH for k in range(31)] + [32 * _CT]
_GRP = [0] + [1] * 12 + [0] * 16 + [1] * 3
_ROWGROUPS = ([(0, 1), (103, 230)], [(1, 103), (230, 256)])

_NT = (((1,), (1,)), ((), ()))


def _rr(*streams):
    streams = [list(s) for s in streams]
    out = []
    while any(streams):
        for s in streams:
            if s:
                out.append(s.pop(0))
    return out


def _merge(bl, al, f):
    gb = [bl[j:j + 2] for j in range(0, len(bl), 2)]
    ga = [al[j:j + 2] for j in range(0, len(al), 2)]
    ne = (int(round(len(bl) * f)) - len(bl)) // 2
    out, k = [], 0
    for j, g in enumerate(gb):
        out += g
        while k < ((j + 1) * ne) // len(gb):
            out += ga[k]
            k += 1
    for g in ga[k:]:
        out += g
    return out


def _schedule(nstep):
    last = nstep - 1

    def blocks(c, i, bs):
        return [((c, i, 2 * b - 1), (c, i, 2 * b) if b < 16 else (c, i + 1, 0)) for b in bs]

    def unit(i, s1, s2):
        return _rr(blocks("k", i, s1), blocks("v", i, s1), blocks("k", i, s2), blocks("v", i, s2))

    ua = lambda i: unit(i, (7, 8, 9, 10), (11, 12, 13, 14))
    ub = lambda i: unit(i, (1, 2, 15, 16), (3, 4, 5, 6))

    first_irr = last - len(_FS)
    visits = [(("k", 0, 0), ("v", 0, 0))] + ua(0)
    npre = len(visits)
    for i in range(last):
        visits += _merge(ub(i), ua(i + 1), _FS[i - first_irr] if i >= first_irr else 2.0)
    visits.append((("k", last, 31), ("v", last, 31)))
    tk, tv = (_rr(blocks(c, last, (1, 2, 15)), blocks(c, last, (3, 4, 5, 6))) for c in "kv")
    nv = 0
    for j, d in enumerate(tk):
        while nv < ((j + 1) * (len(tv) - _VTAIL)) // len(tk):
            visits.append(tv[nv])
            nv += 1
        visits.append(d)
    visits += tv[nv:]
    order = [d for v in visits for d in v]
    assert len(set(order)) == len(order) == nstep * 64

    s0 = order[:len(order) - _QD:2]
    s1 = order[1:len(order) - _QD:2] + order[len(order) - _QD:]
    assert len(s0) == len(s1) - _QD
    pairs = list(zip(s0, s1[_QD:]))

    done = {}
    for pos, (_, i, k) in enumerate(order):
        done[(i, _GRP[k])] = (pos + 1) / 2
    npro = npre + _PY - 32
    prev, t, bursts = npro, 0.0, {}
    for i in range(nstep):
        for u in (0, 1):
            lim = npre + 32 * i + (_PX, _PY)[u]
            if i > first_irr:
                lim = min(lim, int(round(t + _LA_END)))
            lim = len(pairs) if i == last else max(prev, min(lim, len(pairs)))
            bursts[(i, u)] = pairs[prev:lim]
            prev = lim
            t = max(t, done[(i, u)]) + _CU

    rel = lambda i, u: [tuple((c, j - i, k) for c, j, k in p) for p in bursts[(i, u)]]
    regular = [rel(1, 0), rel(1, 1)]
    nloop = 0
    while rel(nloop, 1) == regular[1] and rel(nloop + 1, 0) == regular[0]:
        nloop += 1

    issued = set(s1[:_QD]) | {d for p in pairs[:npro] for d in p}
    nslot = 1 + max(d[1] for d in issued)
    for i in range(nstep):
        for u in (0, 1):
            for p in bursts[(i, u)]:
                issued.update(p)
                nslot = max(nslot, 1 + max(d[1] for d in p) - i)
            assert all((c, i, k) in issued for c in "kv" for k in range(32) if _GRP[k] == u)
    return s0[:npro], s1[:npro + _QD], bursts, regular, nloop, nslot


@jax.jit
def pallas_standalone__mha_block_cached__near_ridge_kernel(
    x: jax.Array,
    k_cache: jax.Array,
    v_cache: jax.Array,
    wq: jax.Array,
    wo: jax.Array,
):
    B, SQ, D = x.shape
    _, H, SK, DH = k_cache.shape
    assert (SK, DH, H * DH) == (2048, 256, 2 * _CT * 128) and D % (8 * _WS) == 0
    bf16, f32 = jnp.bfloat16, jnp.float32
    NSTEP = B * H
    LAST = NSTEP - 1
    TPS = SK // 8 * 2
    SU = SK // 2
    a_tiles = {t for k in range(32) if _GRP[k] == 0 for t in range(_EDGE[k], _EDGE[k + 1])}
    assert all(set(range(2 * lo, 2 * hi)) <= a_tiles for lo, hi in _ROWGROUPS[0])
    pro0, pro1, bursts, regular, nloop, ns = _schedule(NSTEP)

    def kernel_function(x_hbm, k_hbm, v_hbm, wq_hbm, wo_hbm, out_hbm,
                        xbuf, wqbuf, wobuf, kbuf, vbuf, acc, obuf, qbuf, opbuf,
                        sem, osem):

        def kv_copy(kind, step, k):
            src, dst, base = (k_hbm, kbuf, 3) if kind == "k" else (v_hbm, vbuf, 3 + 2 * ns)
            slot = step % ns
            tiles = pl.ds(_EDGE[k], _EDGE[k + 1] - _EDGE[k])
            return pltpu.make_async_copy(
                src.at[step, tiles], dst.at[slot, tiles], sem.at[base + 2 * slot + _GRP[k]])

        def start_pairs(pairs, step0=0):
            for pair in pairs:
                for prio, (kind, step, k) in enumerate(pair):
                    kv_copy(kind, step0 + step, k).start(priority=prio)

        def wait(kind, step, g):
            for k in range(32):
                if _GRP[k] == g:
                    kv_copy(kind, step, k).wait()

        def w_streams(src, dst, s):
            def cp(slab, lo, hi):
                idx = (pl.ds(slab * 8, 8), pl.ds(lo * 128, (hi - lo) * 128))
                return pltpu.make_async_copy(src.at[idx], dst.at[idx], s)

            per = D // 8 // _WS
            streams = []
            for first in range(0, D // 8, per):
                visits = [[]]
                for slab in range(first, first + per):
                    visits[-1].append(cp(slab, 0, _PH))
                    visits.append([cp(slab, _PH, _PH + _CT)])
                    visits.append([cp(slab, _PH + _CT, 2 * _CT)])
                streams.append(visits)
            return streams

        def out_copy(lo, n, s):
            return pltpu.make_async_copy(
                obuf.at[pl.ds(lo, n)], out_hbm.at[pl.ds(lo, n)], osem.at[s])

        xs = []
        for b in range(B):
            for r in range(0, SQ, _XROWS):
                rows = pl.ds(r, min(_XROWS, SQ - r))
                xs.append([pltpu.make_async_copy(x_hbm.at[b, rows], xbuf.at[b, rows], sem.at[0])])
        s0 = sum(_rr(xs[:len(xs) // 2], *w_streams(wq_hbm, wqbuf, sem.at[1])), [])
        s1 = sum(_rr(xs[len(xs) // 2:], *w_streams(wo_hbm, wobuf, sem.at[2])), [])
        s0 += [kv_copy(*d) for d in pro0]
        s1 += [kv_copy(*d) for d in pro1]
        assert len(s0) == len(s1) - _QD
        for c in s1[:_QD]:
            c.start(priority=1)
        for c0, c1 in zip(s0, s1[_QD:]):
            c0.start(priority=0)
            c1.start(priority=1)
        acc[...] = jnp.zeros(acc.shape, f32)
        opbuf[...] = jnp.zeros(opbuf.shape, bf16)
        pltpu.make_async_copy(xbuf, xbuf, sem.at[0]).wait()
        pltpu.make_async_copy(wqbuf, wqbuf, sem.at[1]).wait()
        pltpu.make_async_copy(wobuf, wobuf, sem.at[2]).wait()

        def head_cols(h):
            return pl.ds(h * DH if isinstance(h, int) else pl.multiple_of(h * DH, DH), DH)

        def qproj(i):
            q = jnp.dot(xbuf[i // H], wqbuf[:, head_cols(i % H)], preferred_element_type=f32)
            return (q * (DH ** -0.5)).astype(bf16)

        def oproj(o, h):
            return lax.dot_general(o, wobuf[:, head_cols(h)], _NT, preferred_element_type=f32)

        def load(buf, step, g):
            t = jnp.concatenate(
                [buf[step % ns, pl.ds(2 * lo, 2 * (hi - lo))] for lo, hi in _ROWGROUPS[g]], axis=0)
            t = t.reshape(SU // 8, 2, 8, 128)
            return jnp.concatenate(
                [t[:, 0].reshape(SU, 128), t[:, 1].reshape(SU, 128)], axis=1)

        def scores(k):
            return lax.dot_general(qbuf[...], k, _NT, preferred_element_type=f32)

        def attend(s, v, state=None):
            m = jnp.max(s, axis=-1, keepdims=True)
            if state is not None:
                m = jnp.maximum(state[0], m)
                a = jnp.exp(state[0] - m)
            p = jnp.exp(s - m)
            l = jnp.sum(p, axis=-1, keepdims=True)
            o = jnp.dot(p.astype(bf16), v, preferred_element_type=f32)
            if state is not None:
                l = a * state[1] + l
                o = a * state[2] + o
            return m, l, o

        def step(i, pairs_b, pairs_a, step0):
            h = i % H
            wait("k", i, 0)
            wait("v", i, 0)
            s = scores(load(kbuf, i, 0))
            acc[...] += oproj(opbuf[...], (h + H - 1) % H)
            state = attend(s, load(vbuf, i, 0))
            start_pairs(pairs_b, step0[0])

            @pl.when(jnp.logical_and(h == 0, i > 0))
            def _():
                obuf[i // H - 1] = acc[...].astype(bf16)
                acc[...] = jnp.zeros(acc.shape, f32)

            wait("k", i, 1)
            wait("v", i, 1)
            s = scores(load(kbuf, i, 1))
            qbuf[...] = qproj(i + 1)
            _, l, o = attend(s, load(vbuf, i, 1), state)
            opbuf[...] = (o / l).astype(bf16)
            start_pairs(pairs_a, step0[1])

        qbuf[...] = qproj(0)
        start_pairs(bursts[(0, 0)])

        def body(i, carry):
            step(i, regular[1], regular[0], (i, i + 1))
            return carry

        lax.fori_loop(0, nloop, body, 0)
        for j in range(nloop, LAST):
            step(j, bursts[(j, 1)], bursts[(j + 1, 0)], (0, 0))

        def last_unit(g, state):
            k, v = load(kbuf, LAST, g), load(vbuf, LAST, g)
            sa, sb = scores(k[:SU // 2]), scores(k[SU // 2:])
            return attend(sb, v[SU // 2:], attend(sa, v[:SU // 2], state))

        acc[...] += oproj(opbuf[...], H - 2)
        wait("k", LAST, 0)
        wait("v", LAST, 0)
        state = last_unit(0, None)
        wait("k", LAST, 1)
        out_copy(0, B - 1, 0).start()
        wait("v", LAST, 1)
        _, l, o = last_unit(1, state)
        obuf[B - 1] = (acc[...] + oproj((o / l).astype(bf16), H - 1)).astype(bf16)
        out_copy(B - 1, 1, 1).start()
        out_copy(0, B - 1, 0).wait()
        out_copy(B - 1, 1, 1).wait()

    def tile_view(a):
        a = a.reshape(NSTEP, SK // 8, 8, 2, 128).transpose(0, 1, 3, 2, 4)
        return a.reshape(NSTEP, TPS, 8, 128)

    hbm = pl.BlockSpec(memory_space=pltpu.MemorySpace.HBM)
    return pl.pallas_call(
        kernel_function,
        in_specs=[hbm] * 5,
        out_specs=hbm,
        out_shape=jax.ShapeDtypeStruct((B, SQ, D), x.dtype),
        scratch_shapes=[
            pltpu.VMEM((B, SQ, D), bf16),
            pltpu.VMEM((D, H * DH), bf16),
            pltpu.VMEM((D, H * DH), bf16),
            pltpu.VMEM((ns, TPS, 8, 128), bf16),
            pltpu.VMEM((ns, TPS, 8, 128), bf16),
            pltpu.VMEM((SQ, D), f32),
            pltpu.VMEM((B, SQ, D), bf16),
            pltpu.VMEM((SQ, DH), bf16),
            pltpu.VMEM((SQ, DH), bf16),
            pltpu.SemaphoreType.DMA((3 + 4 * ns,)),
            pltpu.SemaphoreType.DMA((2,)),
        ],
        compiler_params=pltpu.CompilerParams(
            vmem_limit_bytes=48 * 1024 * 1024,
            disable_bounds_checks=True,
            disable_semaphore_checks=True,
        ),
    )(x, tile_view(k_cache), tile_view(v_cache), wq, wo.T)
```

```python
import jax
import jax.numpy as jnp
from jax import lax
import jax.experimental.pallas as pl
import jax.experimental.pallas.tpu as pltpu

_CT = 16
_PH = 13
_QD = 26
_PX, _PY = 40, 56
_LA_END = 28.6
_CU = 13.6
_FS = (1.75, 1.5, 1.25, 1.0, 1.0)
_VTAIL = 6
_WS = 4
_XROWS = 32

_EDGE = [0] + [_CT * k + _PH for k in range(31)] + [32 * _CT]
_GRP = [0] + [1] * 12 + [0] * 16 + [1] * 3
_ROWGROUPS = ([(0, 1), (103, 230)], [(1, 103), (230, 256)])

_NT = (((1,), (1,)), ((), ()))


def _rr(*streams):
    streams = [list(s) for s in streams]
    out = []
    while any(streams):
        for s in streams:
            if s:
                out.append(s.pop(0))
    return out


def _merge(bl, al, f):
    gb = [bl[j:j + 2] for j in range(0, len(bl), 2)]
    ga = [al[j:j + 2] for j in range(0, len(al), 2)]
    ne = (int(round(len(bl) * f)) - len(bl)) // 2
    out, k = [], 0
    for j, g in enumerate(gb):
        out += g
        while k < ((j + 1) * ne) // len(gb):
            out += ga[k]
            k += 1
    for g in ga[k:]:
        out += g
    return out


def _schedule(nstep):
    last = nstep - 1

    def blocks(c, i, bs):
        return [((c, i, 2 * b - 1), (c, i, 2 * b) if b < 16 else (c, i + 1, 0)) for b in bs]

    def unit(i, s1, s2):
        return _rr(blocks("k", i, s1), blocks("v", i, s1), blocks("k", i, s2), blocks("v", i, s2))

    ua = lambda i: unit(i, (7, 8, 9, 10), (11, 12, 13, 14))
    ub = lambda i: unit(i, (1, 2, 15, 16), (3, 4, 5, 6))

    first_irr = last - len(_FS)
    visits = [(("k", 0, 0), ("v", 0, 0))] + ua(0)
    npre = len(visits)
    for i in range(last):
        visits += _merge(ub(i), ua(i + 1), _FS[i - first_irr] if i >= first_irr else 2.0)
    visits.append((("k", last, 31), ("v", last, 31)))
    tk, tv = (_rr(blocks(c, last, (1, 2, 15)), blocks(c, last, (3, 4, 5, 6))) for c in "kv")
    nv = 0
    for j, d in enumerate(tk):
        while nv < ((j + 1) * (len(tv) - _VTAIL)) // len(tk):
            visits.append(tv[nv])
            nv += 1
        visits.append(d)
    visits += tv[nv:]
    order = [d for v in visits for d in v]
    assert len(set(order)) == len(order) == nstep * 64

    s0 = order[:len(order) - _QD:2]
    s1 = order[1:len(order) - _QD:2] + order[len(order) - _QD:]
    assert len(s0) == len(s1) - _QD
    pairs = list(zip(s0, s1[_QD:]))

    done = {}
    for pos, (_, i, k) in enumerate(order):
        done[(i, _GRP[k])] = (pos + 1) / 2
    npro = npre + _PY - 32
    prev, t, bursts = npro, 0.0, {}
    for i in range(nstep):
        for u in (0, 1):
            lim = npre + 32 * i + (_PX, _PY)[u]
            if i > first_irr:
                lim = min(lim, int(round(t + _LA_END)))
            lim = len(pairs) if i == last else max(prev, min(lim, len(pairs)))
            bursts[(i, u)] = pairs[prev:lim]
            prev = lim
            t = max(t, done[(i, u)]) + _CU

    rel = lambda i, u: [tuple((c, j - i, k) for c, j, k in p) for p in bursts[(i, u)]]
    regular = [rel(1, 0), rel(1, 1)]
    nloop = 0
    while rel(nloop, 1) == regular[1] and rel(nloop + 1, 0) == regular[0]:
        nloop += 1

    issued = set(s1[:_QD]) | {d for p in pairs[:npro] for d in p}
    nslot = 1 + max(d[1] for d in issued)
    for i in range(nstep):
        for u in (0, 1):
            for p in bursts[(i, u)]:
                issued.update(p)
                nslot = max(nslot, 1 + max(d[1] for d in p) - i)
            assert all((c, i, k) in issued for c in "kv" for k in range(32) if _GRP[k] == u)
    return s0[:npro], s1[:npro + _QD], bursts, regular, nloop, nslot


@jax.jit
def pallas_standalone__mha_block_cached__near_ridge_kernel(
    x: jax.Array,
    k_cache: jax.Array,
    v_cache: jax.Array,
    wq: jax.Array,
    wo: jax.Array,
):
    B, SQ, D = x.shape
    _, H, SK, DH = k_cache.shape
    assert (SK, DH, H * DH) == (2048, 256, 2 * _CT * 128) and D % (8 * _WS) == 0
    bf16, f32 = jnp.bfloat16, jnp.float32
    NSTEP = B * H
    LAST = NSTEP - 1
    TPS = SK // 8 * 2
    SU = SK // 2
    a_tiles = {t for k in range(32) if _GRP[k] == 0 for t in range(_EDGE[k], _EDGE[k + 1])}
    assert all(set(range(2 * lo, 2 * hi)) <= a_tiles for lo, hi in _ROWGROUPS[0])
    pro0, pro1, bursts, regular, nloop, ns = _schedule(NSTEP)

    def kernel_function(x_hbm, k_hbm, v_hbm, wq_hbm, wo_hbm, out_hbm,
                        xbuf, wqbuf, wobuf, kbuf, vbuf, acc, obuf, qbuf, opbuf,
                        sem, osem):

        def kv_copy(kind, step, k):
            src, dst, base = (k_hbm, kbuf, 3) if kind == "k" else (v_hbm, vbuf, 3 + 2 * ns)
            slot = step % ns
            tiles = pl.ds(_EDGE[k], _EDGE[k + 1] - _EDGE[k])
            return pltpu.make_async_copy(
                src.at[step, tiles], dst.at[slot, tiles], sem.at[base + 2 * slot + _GRP[k]])

        def start_pairs(pairs, step0=0):
            for pair in pairs:
                for prio, (kind, step, k) in enumerate(pair):
                    kv_copy(kind, step0 + step, k).start(priority=prio)

        def wait(kind, step, g):
            for k in range(32):
                if _GRP[k] == g:
                    kv_copy(kind, step, k).wait()

        def w_block(src, dst, s, slab):
            def cp(slab, lo, hi):
                idx = (pl.ds(slab * 8, 8), pl.ds(lo * 128, (hi - lo) * 128))
                return pltpu.make_async_copy(src.at[idx], dst.at[idx], s)

            return cp(slab, _PH, 2 * _CT), cp((slab + 1) % (D // 8), 0, _PH)

        def out_copy(lo, n, s):
            return pltpu.make_async_copy(
                obuf.at[pl.ds(lo, n)], out_hbm.at[pl.ds(lo, n)], osem.at[s])

        xs = []
        for b in range(B):
            for r in range(0, SQ, _XROWS):
                rows = pl.ds(r, min(_XROWS, SQ - r))
                xs.append(pltpu.make_async_copy(x_hbm.at[b, rows], xbuf.at[b, rows], sem.at[0]))
        streams = [zip(xs[:len(xs) // 2], xs[len(xs) // 2:])]
        per = D // 8 // _WS
        for slabs in (range(w * per, (w + 1) * per) for w in range(_WS)):
            streams.append([w_block(wq_hbm, wqbuf, sem.at[1], r) for r in slabs])
            streams.append([w_block(wo_hbm, wobuf, sem.at[2], r)[::-1] for r in slabs])
        visits = _rr(*streams)
        s0 = [v[0] for v in visits] + [kv_copy(*d) for d in pro0]
        s1 = [v[1] for v in visits] + [kv_copy(*d) for d in pro1]
        assert len(s0) == len(s1) - _QD
        for c in s1[:_QD]:
            c.start(priority=1)
        for c0, c1 in zip(s0, s1[_QD:]):
            c0.start(priority=0)
            c1.start(priority=1)
        acc[...] = jnp.zeros(acc.shape, f32)
        opbuf[...] = jnp.zeros(opbuf.shape, bf16)
        pltpu.make_async_copy(xbuf, xbuf, sem.at[0]).wait()
        pltpu.make_async_copy(wqbuf, wqbuf, sem.at[1]).wait()
        pltpu.make_async_copy(wobuf, wobuf, sem.at[2]).wait()

        def head_cols(h):
            return pl.ds(h * DH if isinstance(h, int) else pl.multiple_of(h * DH, DH), DH)

        def qproj(i):
            q = jnp.dot(xbuf[i // H], wqbuf[:, head_cols(i % H)], preferred_element_type=f32)
            return (q * (DH ** -0.5)).astype(bf16)

        def oproj(o, h):
            return lax.dot_general(o, wobuf[:, head_cols(h)], _NT, preferred_element_type=f32)

        def load(buf, step, g):
            t = jnp.concatenate(
                [buf[step % ns, pl.ds(2 * lo, 2 * (hi - lo))] for lo, hi in _ROWGROUPS[g]], axis=0)
            t = t.reshape(SU // 8, 2, 8, 128)
            return jnp.concatenate(
                [t[:, 0].reshape(SU, 128), t[:, 1].reshape(SU, 128)], axis=1)

        def scores(k):
            return lax.dot_general(qbuf[...], k, _NT, preferred_element_type=f32)

        def attend(s, v, state=None):
            m = jnp.max(s, axis=-1, keepdims=True)
            if state is not None:
                m = jnp.maximum(state[0], m)
                a = jnp.exp(state[0] - m)
            p = jnp.exp(s - m)
            l = jnp.sum(p, axis=-1, keepdims=True)
            o = jnp.dot(p.astype(bf16), v, preferred_element_type=f32)
            if state is not None:
                l = a * state[1] + l
                o = a * state[2] + o
            return m, l, o

        def step(i, pairs_b, pairs_a, step0):
            h = i % H
            wait("k", i, 0)
            wait("v", i, 0)
            s = scores(load(kbuf, i, 0))
            acc[...] += oproj(opbuf[...], (h + H - 1) % H)
            state = attend(s, load(vbuf, i, 0))
            start_pairs(pairs_b, step0[0])

            @pl.when(jnp.logical_and(h == 0, i > 0))
            def _():
                obuf[i // H - 1] = acc[...].astype(bf16)
                acc[...] = jnp.zeros(acc.shape, f32)

            wait("k", i, 1)
            wait("v", i, 1)
            s = scores(load(kbuf, i, 1))
            qbuf[...] = qproj(i + 1)
            _, l, o = attend(s, load(vbuf, i, 1), state)
            opbuf[...] = (o / l).astype(bf16)
            start_pairs(pairs_a, step0[1])

        qbuf[...] = qproj(0)
        start_pairs(bursts[(0, 0)])

        def body(i, carry):
            step(i, regular[1], regular[0], (i, i + 1))
            return carry

        lax.fori_loop(0, nloop, body, 0)
        for j in range(nloop, LAST):
            step(j, bursts[(j, 1)], bursts[(j + 1, 0)], (0, 0))

        acc[...] += oproj(opbuf[...], H - 2)
        wait("k", LAST, 0)
        wait("v", LAST, 0)
        k, v = load(kbuf, LAST, 0), load(vbuf, LAST, 0)
        sa, sb = scores(k[:SU // 2]), scores(k[SU // 2:])
        m0, l, o = attend(sb, v[SU // 2:], attend(sa, v[:SU // 2]))
        wait("k", LAST, 1)
        out_copy(0, B - 1, 0).start()
        s = scores(load(kbuf, LAST, 1))
        m = jnp.maximum(m0, jnp.max(s, axis=-1, keepdims=True))
        a = jnp.exp(m0 - m)
        p = jnp.exp(s - m)
        l = a * l + jnp.sum(p, axis=-1, keepdims=True)
        p, o = p.astype(bf16), a * o
        wait("v", LAST, 1)
        o = o + jnp.dot(p, load(vbuf, LAST, 1), preferred_element_type=f32)
        obuf[B - 1] = (acc[...] + oproj((o / l).astype(bf16), H - 1)).astype(bf16)
        out_copy(B - 1, 1, 1).start()
        out_copy(0, B - 1, 0).wait()
        out_copy(B - 1, 1, 1).wait()

    def tile_view(a):
        a = a.reshape(NSTEP, SK // 8, 8, 2, 128).transpose(0, 1, 3, 2, 4)
        return a.reshape(NSTEP, TPS, 8, 128)

    hbm = pl.BlockSpec(memory_space=pltpu.MemorySpace.HBM)
    return pl.pallas_call(
        kernel_function,
        in_specs=[hbm] * 5,
        out_specs=hbm,
        out_shape=jax.ShapeDtypeStruct((B, SQ, D), x.dtype),
        scratch_shapes=[
            pltpu.VMEM((B, SQ, D), bf16),
            pltpu.VMEM((D, H * DH), bf16),
            pltpu.VMEM((D, H * DH), bf16),
            pltpu.VMEM((ns, TPS, 8, 128), bf16),
            pltpu.VMEM((ns, TPS, 8, 128), bf16),
            pltpu.VMEM((SQ, D), f32),
            pltpu.VMEM((B, SQ, D), bf16),
            pltpu.VMEM((SQ, DH), bf16),
            pltpu.VMEM((SQ, DH), bf16),
            pltpu.SemaphoreType.DMA((3 + 4 * ns,)),
            pltpu.SemaphoreType.DMA((2,)),
        ],
        compiler_params=pltpu.CompilerParams(
            vmem_limit_bytes=48 * 1024 * 1024,
            disable_bounds_checks=True,
            disable_semaphore_checks=True,
        ),
    )(x, tile_view(k_cache), tile_view(v_cache), wq, wo.T)
```

```python
import jax
import jax.numpy as jnp
from jax import lax
import jax.experimental.pallas as pl
import jax.experimental.pallas.tpu as pltpu

_CT = 16
_PH = 13
_QD = 26
_PX, _PY = 40, 56
_LA_END = 28.6
_CU = 13.6
_FS = (1.75, 1.5, 1.25, 1.0, 1.0)
_VTAIL = 6
_WS = 4
_X0 = 24

_EDGE = [0] + [_CT * k + _PH for k in range(31)] + [32 * _CT]
_GRP = [0] + [1] * 12 + [0] * 16 + [1] * 3
_ROWGROUPS = ([(0, 1), (103, 230)], [(1, 103), (230, 256)])

_NT = (((1,), (1,)), ((), ()))


def _rr(*streams):
    streams = [list(s) for s in streams]
    out = []
    while any(streams):
        for s in streams:
            if s:
                out.append(s.pop(0))
    return out


def _merge(bl, al, f):
    gb = [bl[j:j + 2] for j in range(0, len(bl), 2)]
    ga = [al[j:j + 2] for j in range(0, len(al), 2)]
    ne = (int(round(len(bl) * f)) - len(bl)) // 2
    out, k = [], 0
    for j, g in enumerate(gb):
        out += g
        while k < ((j + 1) * ne) // len(gb):
            out += ga[k]
            k += 1
    for g in ga[k:]:
        out += g
    return out


def _schedule(nstep):
    last = nstep - 1

    def blocks(c, i, bs):
        return [((c, i, 2 * b - 1), (c, i, 2 * b) if b < 16 else (c, i + 1, 0)) for b in bs]

    def unit(i, s1, s2):
        return _rr(blocks("k", i, s1), blocks("v", i, s1), blocks("k", i, s2), blocks("v", i, s2))

    ua = lambda i: unit(i, (7, 8, 9, 10), (11, 12, 13, 14))
    ub = lambda i: unit(i, (1, 2, 15, 16), (3, 4, 5, 6))

    first_irr = last - len(_FS)
    visits = [(("k", 0, 0), ("v", 0, 0))] + ua(0)
    npre = len(visits)
    for i in range(last):
        visits += _merge(ub(i), ua(i + 1), _FS[i - first_irr] if i >= first_irr else 2.0)
    visits.append((("k", last, 31), ("v", last, 31)))
    tk, tv = (_rr(blocks(c, last, (1, 2, 15)), blocks(c, last, (3, 4, 5, 6))) for c in "kv")
    nv = 0
    for j, d in enumerate(tk):
        while nv < ((j + 1) * (len(tv) - _VTAIL)) // len(tk):
            visits.append(tv[nv])
            nv += 1
        visits.append(d)
    visits += tv[nv:]
    order = [d for v in visits for d in v]
    assert len(set(order)) == len(order) == nstep * 64

    s0 = order[:len(order) - _QD:2]
    s1 = order[1:len(order) - _QD:2] + order[len(order) - _QD:]
    assert len(s0) == len(s1) - _QD
    pairs = list(zip(s0, s1[_QD:]))

    done = {}
    for pos, (_, i, k) in enumerate(order):
        done[(i, _GRP[k])] = (pos + 1) / 2
    npro = npre + _PY - 32
    prev, t, bursts = npro, 0.0, {}
    for i in range(nstep):
        for u in (0, 1):
            lim = npre + 32 * i + (_PX, _PY)[u]
            if i > first_irr:
                lim = min(lim, int(round(t + _LA_END)))
            lim = len(pairs) if i == last else max(prev, min(lim, len(pairs)))
            bursts[(i, u)] = pairs[prev:lim]
            prev = lim
            t = max(t, done[(i, u)]) + _CU

    rel = lambda i, u: [tuple((c, j - i, k) for c, j, k in p) for p in bursts[(i, u)]]
    regular = [rel(1, 0), rel(1, 1)]
    nloop = 0
    while rel(nloop, 1) == regular[1] and rel(nloop + 1, 0) == regular[0]:
        nloop += 1

    issued = set(s1[:_QD]) | {d for p in pairs[:npro] for d in p}
    nslot = 1 + max(d[1] for d in issued)
    for i in range(nstep):
        for u in (0, 1):
            for p in bursts[(i, u)]:
                issued.update(p)
                nslot = max(nslot, 1 + max(d[1] for d in p) - i)
            assert all((c, i, k) in issued for c in "kv" for k in range(32) if _GRP[k] == u)
    return s0[:npro], s1[:npro + _QD], bursts, regular, nloop, nslot


@jax.jit
def pallas_standalone__mha_block_cached__near_ridge_kernel(
    x: jax.Array,
    k_cache: jax.Array,
    v_cache: jax.Array,
    wq: jax.Array,
    wo: jax.Array,
):
    B, SQ, D = x.shape
    _, H, SK, DH = k_cache.shape
    assert (SK, DH, H * DH) == (2048, 256, 2 * _CT * 128) and D % (8 * _WS) == 0 and SQ % 16 == 0
    bf16, f32 = jnp.bfloat16, jnp.float32
    NSTEP = B * H
    LAST = NSTEP - 1
    TPS = SK // 8 * 2
    SU = SK // 2
    a_tiles = {t for k in range(32) if _GRP[k] == 0 for t in range(_EDGE[k], _EDGE[k + 1])}
    assert all(set(range(2 * lo, 2 * hi)) <= a_tiles for lo, hi in _ROWGROUPS[0])
    pro0, pro1, bursts, regular, nloop, ns = _schedule(NSTEP)

    def kernel_function(x_hbm, k_hbm, v_hbm, wq_hbm, wo_hbm, out_hbm,
                        xbuf, wqbuf, wobuf, kbuf, vbuf, acc, obuf, qbuf, opbuf,
                        sem, osem):

        def kv_copy(kind, step, k):
            src, dst, base = (k_hbm, kbuf, 3) if kind == "k" else (v_hbm, vbuf, 3 + 2 * ns)
            slot = step % ns
            tiles = pl.ds(_EDGE[k], _EDGE[k + 1] - _EDGE[k])
            return pltpu.make_async_copy(
                src.at[step, tiles], dst.at[slot, tiles], sem.at[base + 2 * slot + _GRP[k]])

        def start_pairs(pairs, step0=0):
            for pair in pairs:
                for prio, (kind, step, k) in enumerate(pair):
                    kv_copy(kind, step0 + step, k).start(priority=prio)

        def wait(kind, step, g):
            for k in range(32):
                if _GRP[k] == g:
                    kv_copy(kind, step, k).wait()

        def w_block(src, dst, s, slab):
            def cp(slab, lo, hi):
                idx = (pl.ds(slab * 8, 8), pl.ds(lo * 128, (hi - lo) * 128))
                return pltpu.make_async_copy(src.at[idx], dst.at[idx], s)

            return cp(slab, _PH, 2 * _CT), cp((slab + 1) % (D // 8), 0, _PH)

        def out_copy(lo, n, s):
            return pltpu.make_async_copy(
                obuf.at[pl.ds(lo, n)], out_hbm.at[pl.ds(lo, n)], osem.at[s])

        def x_copy(lo, hi):
            rows = pl.ds(lo, hi - lo)
            return pltpu.make_async_copy(x_hbm.at[rows], xbuf.at[rows], sem.at[0])

        cuts = range(_X0, B * SQ, 64)
        xv = [(x_copy(r, r + 32), x_copy(r + 32, r + 64)) for r in cuts[:-1]]
        xv.append((x_copy(cuts[-1], B * SQ), x_copy(0, _X0)))
        streams = [xv[:len(xv) // 2], xv[len(xv) // 2:]]
        per = D // 8 // _WS
        for slabs in (range(w * per, (w + 1) * per) for w in range(_WS)):
            streams.append([w_block(wq_hbm, wqbuf, sem.at[1], r) for r in slabs])
            streams.append([w_block(wo_hbm, wobuf, sem.at[2], r)[::-1] for r in slabs])
        visits = _rr(*streams)
        s0 = [v[0] for v in visits] + [kv_copy(*d) for d in pro0]
        s1 = [v[1] for v in visits] + [kv_copy(*d) for d in pro1]
        assert len(s0) == len(s1) - _QD
        for c in s1[:_QD]:
            c.start(priority=1)
        for c0, c1 in zip(s0, s1[_QD:]):
            c0.start(priority=0)
            c1.start(priority=1)
        acc[...] = jnp.zeros(acc.shape, f32)
        opbuf[...] = jnp.zeros(opbuf.shape, bf16)
        pltpu.make_async_copy(xbuf, xbuf, sem.at[0]).wait()
        pltpu.make_async_copy(wqbuf, wqbuf, sem.at[1]).wait()
        pltpu.make_async_copy(wobuf, wobuf, sem.at[2]).wait()

        def block(j, size, align):
            return pl.ds(j * size if isinstance(j, int) else pl.multiple_of(j * size, align), size)

        def qproj(i):
            q = jnp.dot(xbuf[block(i // H, SQ, 16)], wqbuf[:, block(i % H, DH, DH)],
                        preferred_element_type=f32)
            return (q * (DH ** -0.5)).astype(bf16)

        def oproj(o, h):
            return lax.dot_general(o, wobuf[:, block(h, DH, DH)], _NT, preferred_element_type=f32)

        def load(buf, step, g):
            t = jnp.concatenate(
                [buf[step % ns, pl.ds(2 * lo, 2 * (hi - lo))] for lo, hi in _ROWGROUPS[g]], axis=0)
            t = t.reshape(SU // 8, 2, 8, 128)
            return jnp.concatenate(
                [t[:, 0].reshape(SU, 128), t[:, 1].reshape(SU, 128)], axis=1)

        def scores(k):
            return lax.dot_general(qbuf[...], k, _NT, preferred_element_type=f32)

        def attend(s, v, state=None):
            m = jnp.max(s, axis=-1, keepdims=True)
            if state is not None:
                m = jnp.maximum(state[0], m)
                a = jnp.exp(state[0] - m)
            p = jnp.exp(s - m)
            l = jnp.sum(p, axis=-1, keepdims=True)
            o = jnp.dot(p.astype(bf16), v, preferred_element_type=f32)
            if state is not None:
                l = a * state[1] + l
                o = a * state[2] + o
            return m, l, o

        def step(i, pairs_b, pairs_a, step0):
            h = i % H
            wait("k", i, 0)
            wait("v", i, 0)
            s = scores(load(kbuf, i, 0))
            acc[...] += oproj(opbuf[...], (h + H - 1) % H)
            state = attend(s, load(vbuf, i, 0))
            start_pairs(pairs_b, step0[0])

            def flush():
                obuf[i // H - 1] = acc[...].astype(bf16)
                acc[...] = jnp.zeros(acc.shape, f32)

            if not isinstance(i, int):
                pl.when(jnp.logical_and(h == 0, i > 0))(flush)
            elif h == 0:
                flush()

            wait("k", i, 1)
            wait("v", i, 1)
            s = scores(load(kbuf, i, 1))
            qbuf[...] = qproj(i + 1)
            _, l, o = attend(s, load(vbuf, i, 1), state)
            opbuf[...] = (o / l).astype(bf16)
            start_pairs(pairs_a, step0[1])

        qbuf[...] = qproj(0)
        start_pairs(bursts[(0, 0)])

        def body(i, carry):
            step(i, regular[1], regular[0], (i, i + 1))
            return carry

        lax.fori_loop(0, nloop, body, 0)
        for j in range(nloop, LAST):
            step(j, bursts[(j, 1)], bursts[(j + 1, 0)], (0, 0))

        acc[...] += oproj(opbuf[...], H - 2)
        wait("k", LAST, 0)
        wait("v", LAST, 0)
        k, v = load(kbuf, LAST, 0), load(vbuf, LAST, 0)
        sa, sb = scores(k[:SU // 2]), scores(k[SU // 2:])
        m0, l, o = attend(sb, v[SU // 2:], attend(sa, v[:SU // 2]))
        wait("k", LAST, 1)
        out_copy(0, B - 1, 0).start()
        s = scores(load(kbuf, LAST, 1))
        m = jnp.maximum(m0, jnp.max(s, axis=-1, keepdims=True))
        a = jnp.exp(m0 - m)
        p = jnp.exp(s - m)
        l = a * l + jnp.sum(p, axis=-1, keepdims=True)
        p, o = p.astype(bf16), a * o
        wait("v", LAST, 1)
        o = o + jnp.dot(p, load(vbuf, LAST, 1), preferred_element_type=f32)
        obuf[B - 1] = (acc[...] + oproj((o / l).astype(bf16), H - 1)).astype(bf16)
        out_copy(B - 1, 1, 1).start()
        out_copy(0, B - 1, 0).wait()
        out_copy(B - 1, 1, 1).wait()

    def tile_view(a):
        a = a.reshape(NSTEP, SK // 8, 8, 2, 128).transpose(0, 1, 3, 2, 4)
        return a.reshape(NSTEP, TPS, 8, 128)

    hbm = pl.BlockSpec(memory_space=pltpu.MemorySpace.HBM)
    return pl.pallas_call(
        kernel_function,
        in_specs=[hbm] * 5,
        out_specs=hbm,
        out_shape=jax.ShapeDtypeStruct((B, SQ, D), x.dtype),
        scratch_shapes=[
            pltpu.VMEM((B * SQ, D), bf16),
            pltpu.VMEM((D, H * DH), bf16),
            pltpu.VMEM((D, H * DH), bf16),
            pltpu.VMEM((ns, TPS, 8, 128), bf16),
            pltpu.VMEM((ns, TPS, 8, 128), bf16),
            pltpu.VMEM((SQ, D), f32),
            pltpu.VMEM((B, SQ, D), bf16),
            pltpu.VMEM((SQ, DH), bf16),
            pltpu.VMEM((SQ, DH), bf16),
            pltpu.SemaphoreType.DMA((3 + 4 * ns,)),
            pltpu.SemaphoreType.DMA((2,)),
        ],
        compiler_params=pltpu.CompilerParams(
            vmem_limit_bytes=48 * 1024 * 1024,
            disable_bounds_checks=True,
            disable_semaphore_checks=True,
        ),
    )(x.reshape(B * SQ, D), tile_view(k_cache), tile_view(v_cache), wq, wo.T)
```
